```python
import jax
import jax.numpy as jnp

def _softmax(x, axis=-1):
    return jax.nn.softmax(x, axis=axis)

def _gelu(x):
    return jax.nn.gelu(x, approximate=True)

def _silu(x):
    return jax.nn.silu(x)

def _sigmoid(x):
    return jax.nn.sigmoid(x)

def _layernorm(x, axis=-1, eps=1e-05):
    m = jnp.mean(x, axis=axis, keepdims=True)
    v = jnp.var(x, axis=axis, keepdims=True)
    return (x - m) / jnp.sqrt(v + eps)

def _scatter_add(tgt, idx, src, axis=0):
    return tgt.at[idx].add(src)

def _segment_sum(src, seg, n):
    return jax.ops.segment_sum(src, seg, n)

class _Rng:

    def __init__(self, key):
        self._k = key

    def _next(self):
        self._k, sub = jax.random.split(self._k)
        return sub

    def normal(self, shape):
        return jax.random.normal(self._next(), shape, dtype=jnp.bfloat16)

    def randint(self, lo, hi, shape):
        return jax.random.randint(self._next(), shape, lo, hi, dtype=jnp.int32)

    def uniform(self, shape, lo=0.0, hi=1.0):
        return jax.random.uniform(self._next(), shape, jnp.bfloat16, lo, hi)

    def permutation(self, n):
        return jax.random.permutation(self._next(), n)
kernel_name = 'adaLN_cond__sliding_block_cached__mixer_s_mlp__decode'

def setup_inputs():
    _rng = _Rng(jax.random.key(int.from_bytes(__import__("os").urandom(4), "little")))
    _w = lambda a: (lambda t: t.astype(jnp.bfloat16) if jnp.issubdtype(t.dtype, jnp.floating) else t)(jnp.asarray(a))

    def _A_setup():
        B, Sq, D = (1, 1, 448)
        Hq, Hkv, Sk, Dh = (16, 8, 65536, 256)
        assert Hq % Hkv == 0, (Hq, Hkv)
        return {'x': _w((lambda *s: _rng.normal(s) * 0.05)(B, Sq, D)), 'k_cache': _w((lambda *s: _rng.normal(s) * 0.05)(B, Hkv, Sk, Dh)), 'v_cache': _w((lambda *s: _rng.normal(s) * 0.05)(B, Hkv, Sk, Dh)), 'wq': _w((lambda *s: _rng.normal(s) * 0.05)(D, Hq * Dh) * D ** (-0.5)), 'wo': _w((lambda *s: _rng.normal(s) * 0.05)(Hq * Dh, D) * (Hq * Dh) ** (-0.5))}
    _A_in = _A_setup()

    def _B_setup():
        B, S, D, F = (1, 1, 448, 1792)
        return {'x': _w((lambda *s: _rng.normal(s) * 0.05)(B, S, D)), 'w1': _w((lambda *s: _rng.normal(s) * 0.05)(D, D) * D ** (-0.5)), 'w2': _w((lambda *s: _rng.normal(s) * 0.05)(D, D) * D ** (-0.5)), 'w3': _w((lambda *s: _rng.normal(s) * 0.05)(D, F) * D ** (-0.5)), 'w4': _w((lambda *s: _rng.normal(s) * 0.05)(F, D) * F ** (-0.5))}
    _B_in = _B_setup()
    return {'A_x': _A_in['x'], 'A_k_cache': _A_in['k_cache'], 'A_v_cache': _A_in['v_cache'], 'A_wq': _A_in['wq'], 'A_wo': _A_in['wo'], 'B_x': _B_in['x'], 'B_w1': _B_in['w1'], 'B_w2': _B_in['w2'], 'B_w3': _B_in['w3'], 'B_w4': _B_in['w4'], 'c': _w((lambda *s: _rng.normal(s) * 0.05)(1, 448)), 'w_mod': _w((lambda *s: _rng.normal(s) * 0.05)(448, 6 * 448) * 448 ** (-0.5))}

def reference(A_x, A_k_cache, A_v_cache, A_wq, A_wo, B_x, B_w1, B_w2, B_w3, B_w4, c, w_mod):

    def _A_ref(x, k_cache, v_cache, wq, wo):
        B, Sq, D = x.shape
        Hq, Dh = (16, 256)
        Hkv, Sk = (k_cache.shape[1], k_cache.shape[2])
        W = min(4096, max(256, Sk // 4))
        rep = Hq // Hkv
        q = (lambda x, *d: x.transpose(*d))((x @ wq).reshape(B, Sq, Hq, Dh), 0, 2, 1, 3)
        k = jnp.repeat(k_cache[:, :, Sk - W:, :], rep, axis=1)
        v = jnp.repeat(v_cache[:, :, Sk - W:, :], rep, axis=1)
        scores = jnp.einsum('bhqd,bhkd->bhqk', q, k) * Dh ** (-0.5)
        p = _softmax(scores, axis=-1)
        o = jnp.einsum('bhqk,bhkd->bhqd', p, v)
        return (lambda x, *d: x.transpose(*d))(o, 0, 2, 1, 3).reshape(B, Sq, Hq * Dh) @ wo

    def _B_ref(x, w1, w2, w3, w4):
        B, S, D = x.shape
        h = _gelu(_layernorm(x, axis=-1) @ w1)
        c = D // 4
        g0 = jnp.pad(h[:, :, 0 * c:1 * c], ((0, 0), (1, 0), (0, 0)))[:, :S, :]
        g1 = jnp.pad(h[:, :, 1 * c:2 * c], ((0, 0), (0, 1), (0, 0)))[:, 1:, :]
        g2 = jnp.pad(h[:, :, 2 * c:3 * c], ((0, 0), (2, 0), (0, 0)))[:, :S, :]
        g3 = jnp.pad(h[:, :, 3 * c:], ((0, 0), (0, 2), (0, 0)))[:, 2:, :]
        hs = jnp.concatenate([g0, g1, g2, g3], axis=-1) @ w2
        x1 = x + hs
        h2 = _gelu(_layernorm(x1, axis=-1) @ w3) @ w4
        return x1 + h2
    x = A_x
    mod = (_silu(c) @ w_mod).reshape(c.shape[0], 6, 1, -1)
    sa, ca, ga, sb, cb, gb = (mod[:, 0].copy(), mod[:, 1].copy(), mod[:, 2].copy(), mod[:, 3].copy(), mod[:, 4].copy(), mod[:, 5].copy())
    h = _layernorm(x, axis=-1) * (1 + ca) + sa
    x = x + ga * _A_ref(h, A_k_cache, A_v_cache, A_wq, A_wo)
    h = _layernorm(x, axis=-1) * (1 + cb) + sb
    x = x + gb * _B_ref(h, B_w1, B_w2, B_w3, B_w4)
    return x
```

```python
import jax
import jax.numpy as jnp
from jax import lax
from jax.experimental import pallas as pl
from jax.experimental.pallas import tpu as pltpu

D, F = 448, 1792
HQ, HKV, DH = 16, 8, 256
EPS = 1e-5
ROWS = 8
STEP = 32
BLOCK = 512
AHEAD = 26
TILE_ROWS = D // 8
GATE = 2304
BF16, F32 = jnp.bfloat16, jnp.float32
CFG = dict(lag=0, korder=(0, 1, 2, 3), vorder=(2, 3, 0, 1), swq=45, swo=45, swm=13, sw3=17, tail=0,
           w4=((64, 128), (192, 128), (320, 128), (0, 64)), gate=(0, 12, 18, 22, 25, 28), at={}, extra=0, early=12, hold=4, order=((0, 2), (1,), (3,)))

S_X, S_C, S_WM, S_WQ, S_WO, S_W3, S_V, S_K, S_W4, S_GATE = 0, 1, 2, 3, 4, 5, 6, 7, 15, 21


def _layernorm(x):
    d = x - jnp.sum(x, axis=-1, keepdims=True) * (1.0 / D)
    return d * lax.rsqrt(jnp.sum(d * d, axis=-1, keepdims=True) * (1.0 / D) + EPS)


def _dot(a, b):
    return lax.dot_general(a, b, (((1,), (0,)), ((), ())), preferred_element_type=F32)


def _dot_t(a, b):
    return lax.dot_general(a, b, (((1,), (1,)), ((), ())), preferred_element_type=F32)


def _ds(start, size):
    return pl.ds(start if isinstance(start, int) else pl.multiple_of(start, size), size)


def _lanes(x, op):
    out = x[:, :128]
    for t in range(128, x.shape[1], 128):
        out = op(out, x[:, t:t + 128])
    return out


def _merge(a, b):
    order = sorted([((i + 0.5) / len(a), 0, i) for i in range(len(a))] + [((i + 0.5) / len(b), 1, i) for i in range(len(b))])
    return [(a, b)[which][i] for _, which, i in order]


def _kernel(x_hbm, c_hbm, wm_hbm, wq_hbm, k_hbm, v_hbm, wo_hbm, w3_hbm, w4_hbm, out_hbm,
            x_ref, c_ref, wm_ref, gate_ref, wq_ref, k_ref, v_ref, wo_ref, w3_ref, w4_ref,
            q_ref, s_ref, max_ref, ctx_ref, mod_ref, cond_ref, last_ref, out_ref, sems, *, cfg):
    steps = k_ref.shape[0]
    window = steps * STEP
    first_key = k_hbm.shape[2] - window
    per_block = BLOCK // STEP

    def cache(hbm, ref, sem, order):
        def copy(j, g):
            return pltpu.make_async_copy(hbm.at[:, order[g], _ds(first_key + j * STEP, STEP)], ref.at[j, order[g]], sems.at[sem(j)])
        return copy

    def streams(hbm, ref, sem, n, cuts):
        spots = [(slice(None), pl.ds(row, 8), pl.ds(128 * lo, 128 * (hi - lo)))
                 for row in range(0, D // n, 8) for lo, hi in zip(cuts[:-1], cuts[1:])]
        return [pltpu.make_async_copy(hbm.at[at], ref.at[at], sems.at[sem]) for at in spots]

    keys = cache(k_hbm, k_ref, lambda j: S_K + j // per_block, cfg['korder'])
    values = cache(v_hbm, v_ref, lambda j: S_V, cfg['vorder'])
    wq, wo = streams(wq_hbm, wq_ref, S_WQ, 4, range(0, 33, 4)), streams(wo_hbm, wo_ref, S_WO, 4, range(0, 33, 4))
    wm = streams(wm_hbm, wm_ref, S_WM, 4, (0, 5, 9, 14, 18))
    w3 = streams(w3_hbm, w3_ref, S_W3, 4, (0, 4, 8, 11, 14))
    w4 = [[pltpu.make_async_copy(w4_hbm.at[pl.ds(row, 8)], w4_ref.at[pl.ds(row, 8)], sems.at[S_W4 + i])
           for row in range(r0, r0 + n, 8)] for i, (r0, n) in enumerate(cfg['w4'])]
    groups = list(zip(cfg['gate'][:-1], cfg['gate'][1:]))
    gate = [pltpu.make_async_copy(wm_hbm.at[j // 7, pl.ds(j % 7 * 16, 16), pl.ds(GATE, 6 * D - GATE)], gate_ref.at[pl.ds(16 * j, 16)],
                                  sems.at[S_GATE + i]) for i, (lo, hi) in enumerate(groups) for j in range(lo, hi)]
    small = [pltpu.make_async_copy(c_hbm, c_ref, sems.at[S_C]), pltpu.make_async_copy(x_hbm, x_ref, sems.at[S_X])]

    def landed(ref, sem):
        pltpu.make_async_copy(ref, ref, sems.at[sem]).wait()

    even = (lax.broadcasted_iota(jnp.int32, (ROWS, DH), 0) & 1) == 0
    live = {}

    def condition():
        for copy in small:
            copy.wait()
        landed(wm_ref, S_WM)
        c = jnp.broadcast_to(c_ref[...].astype(F32), (ROWS, D))
        c = (c * jax.nn.sigmoid(c)).astype(BF16)
        mod = _dot(c, wm_ref[...].reshape(D, GATE))
        for g in range(5):
            mod_ref[g] = mod[:, g * D:(g + 1) * D]
        mod_ref[5, :, :GATE - 5 * D] = mod[:, 5 * D:]
        wide = jnp.concatenate([c.astype(F32), jnp.zeros((ROWS, 512 - D), F32)], axis=1)
        cond_ref[...] = jnp.concatenate([wide] * (128 // ROWS), axis=0).T

    def queries():
        landed(wq_ref, S_WQ)
        x = jnp.broadcast_to(x_ref[0].astype(F32), (ROWS, D))
        h = (_layernorm(x) * (1.0 + mod_ref[1]) + mod_ref[0]).astype(BF16)
        q = _dot(h, wq_ref[...].reshape(D, HQ * DH)) * DH ** -0.5
        for i in range(HKV):
            q_ref[i] = jnp.where(even, q[:, 2 * i * DH:(2 * i + 1) * DH], q[:, (2 * i + 1) * DH:(2 * i + 2) * DH])
            max_ref[i] = jnp.full((ROWS, 128), -jnp.inf, F32)

    def scores(b):
        rows = pl.ds(b * per_block, per_block)
        landed(k_ref.at[rows], S_K + b)
        for h in range(HKV):
            s = _dot_t(q_ref[h].astype(BF16), k_ref[rows, h % 4, h // 4].reshape(BLOCK, DH))
            s_ref[h, :, _ds(b * BLOCK, BLOCK)] = s
            max_ref[h] = jnp.maximum(max_ref[h], _lanes(s, jnp.maximum))

    def context(lo, hi):
        if lo == 0:
            landed(v_ref, S_V)

        def body(h, carry):
            p = jnp.exp(s_ref[h] - jnp.max(max_ref[h], axis=-1, keepdims=True))
            o = _dot(p.astype(BF16), v_ref[:, h & 3, h >> 2].reshape(window, DH))
            o = o / jnp.sum(_lanes(p, jnp.add), axis=-1, keepdims=True)
            ctx_ref[:, _ds(2 * h * DH, 2 * DH)] = jnp.concatenate([jnp.where(even, o, 0.0), jnp.where(even, 0.0, o)], axis=1)
            return carry
        lax.fori_loop(lo, hi, body, None)

    def project(part):
        if part == 0:
            landed(wo_ref, S_WO)

        def body(i, attn):
            cols = _ds(i * 1024, 1024)
            return attn + _dot_t(ctx_ref[:, cols].astype(BF16), wo_ref[:, :, cols].reshape(D, 1024))
        live['attn'] = lax.fori_loop(2 * part, 2 * part + 2, body, live['attn'] if part else jnp.zeros((ROWS, D), F32))

    def residual():
        attn = live['attn'] + pltpu.roll(live['attn'], 1, 0)
        x = jnp.broadcast_to(x_ref[0].astype(F32), (ROWS, D)) + mod_ref[2] * attn
        h = _layernorm(x) * (1.0 + mod_ref[4]) + mod_ref[3]
        live['normed'] = _layernorm(h).astype(BF16)
        for i, v in enumerate((x, h)):
            last_ref[i] = jnp.concatenate([v[:, 64:], v[:, :128]], axis=1)

    if cfg.get('dry'):
        condition = lambda: ([c.wait() for c in small], landed(wm_ref, S_WM))
        queries = lambda: landed(wq_ref, S_WQ)
        scores = lambda b: landed(k_ref.at[pl.ds(b * per_block, per_block)], S_K + b)
        context = lambda lo, hi: landed(v_ref, S_V) if lo == 0 else None
        project = lambda part: landed(wo_ref, S_WO) if part == 0 else None
        residual = lambda: live.update(normed=jnp.zeros((ROWS, D), BF16))
    front = _merge(wm, wq)
    early, hold = cfg.get('early', 24), cfg.get('hold', 0)
    back = _merge(wo, w3[:early]) + _merge(w3[early:], _merge(w4[0], w4[2])[:cfg.get('mid', 16)]) + _merge(w4[0], w4[2])[cfg.get('mid', 16):] + _merge(w4[1], w4[3][:8 - hold]) + w4[3][8 - hold:]
    n_front, n_cache = len(front) // 2, 4 * steps
    lag = cfg['lag']
    spare = len(gate) - AHEAD - cfg['extra']

    def deal(copies, n):
        pick = set(i * len(copies) // n for i in range(n))
        return [c for i, c in enumerate(copies) if i in pick], [c for i, c in enumerate(copies) if i not in pick]
    front1, front0 = deal(front, n_front + lag)
    back1, back0 = deal(back, (len(back) - spare) // 2 - lag)
    back1 += gate

    def first(i):
        i -= len(front1)
        return front1[i] if i < 0 else values(i // 4, i % 4) if i < n_cache else back1[i - n_cache]

    def second(i):
        i -= len(front0)
        return front0[i] if i < 0 else keys(i // 4, i % 4) if i < n_cache else back0[i - n_cache]

    total = len(front0) + n_cache + len(back0)
    loop_lo = len(front0) + 64

    def pairs(lo, hi, work):
        for i in range(lo, hi):
            if i in work:
                work[i]()
            first(AHEAD + i).start(priority=1)
            second(i).start(priority=0)

    at = dict(cond=20, q=40, s6=0, s7=30, c0=36, c1=46, c2=56, c3=66, p0=89, p1=96, r=103)
    at.update(cfg['at'])
    for i in range(AHEAD):
        first(i).start(priority=1)
    for copy in small:
        copy.start(priority=0)
    pairs(0, loop_lo, {len(front0) + at['cond']: condition, len(front0) + at['q']: queries})

    shift = loop_lo + AHEAD - len(front1) - 64

    def block(b, carry):
        for i in range(64):
            if i == 40:
                scores(b - 1)
            values(b * per_block + (i + shift) // 4, (i + shift) % 4).start(priority=1)
            keys(b * per_block + i // 4, i % 4).start(priority=0)
        return carry
    blocks = window // BLOCK
    lax.fori_loop(1, blocks - 1, block, None)

    end = len(front0) + n_cache
    work = {end - 24: lambda: scores(blocks - 2), end + at['s7']: lambda: scores(blocks - 1), end + at['r']: residual}
    for i in range(4):
        work[end + at['c%d' % i]] = lambda i=i: context(2 * i, 2 * i + 2)
    for i in range(2):
        work[end + at['p%d' % i]] = lambda i=i: project(i)
    assert len(work) == 9
    pairs(end - 64, total, work)
    for i in range(AHEAD + total, len(front1) + n_cache + len(back1)):
        first(i).start(priority=1)
    for i in sorted(work):
        if i >= total:
            work[i]()

    landed(w3_ref, S_W3)
    hidden = jax.nn.gelu(_dot(live['normed'], w3_ref[...].reshape(D, F)), approximate=True).astype(BF16)
    y = [None] * 4
    acc = [None] * 3
    for batch in cfg.get('order', ((0, 2), (1, 3))) + tuple((4 + i,) for i in range(len(groups))):
        for i in batch:
            if i < 4:
                landed(w4_ref.at[pl.ds(*cfg['w4'][i])], S_W4 + i)
            else:
                lo, hi = groups[i - 4]
                landed(gate_ref.at[pl.ds(16 * lo, 16 * (hi - lo))], S_GATE + i - 4)
        for i in batch:
            if i < 4:
                r0, n = cfg['w4'][i]
                y[i] = last_ref[1, :, 128 * i:128 * i + n] + (0.0 if cfg.get('dry') == 2 else _dot_t(hidden, w4_ref[r0:r0 + n, :]))
                continue
            for j in range(*groups[i - 4]):
                for t in range(3):
                    w = gate_ref[16 * j:16 * j + 16, 128 * t:128 * t + 128].astype(F32) * cond_ref[16 * j:16 * j + 16, :]
                    w = w[:ROWS] + w[ROWS:]
                    acc[t] = w if acc[t] is None else acc[t] + w
    head = last_ref[0, :, 384:448] + mod_ref[5, :, :64] * y[3]
    turned = [jnp.concatenate([head, jnp.zeros_like(head)], axis=1)]
    for t in range(3):
        for step in (4, 2, 1):
            acc[t] = acc[t] + pltpu.roll(acc[t], step, 0)
        turned.append(pltpu.roll(last_ref[0, :, 128 * t:128 * t + 128] + acc[t] * y[t], 0 if cfg.get('norot') else 64, 1))
    low = lax.broadcasted_iota(jnp.int32, (ROWS, 128), 1) < 64
    tiles = [jnp.where(low, turned[t], turned[t + 1]) for t in range(3)] + [turned[3][:, :64]]
    out_ref[0] = jnp.concatenate(tiles, axis=1)[:1].astype(BF16)
    store = pltpu.make_async_copy(out_ref, out_hbm, sems.at[S_X])
    store.start()
    store.wait()


def build(interpret=False, **changes):
    cfg = dict(CFG, **changes)

    @jax.jit
    def run(A_x, A_k_cache, A_v_cache, A_wq, A_wo, B_x, B_w1, B_w2, B_w3, B_w4, c, w_mod):
        keys = A_k_cache.shape[2]
        window = min(4096, max(256, keys // 4))
        assert A_x.shape == (1, 1, D) and A_k_cache.shape == (1, HKV, keys, DH) and window == 4096
        hbm = pl.BlockSpec(memory_space=pltpu.HBM)
        return pl.pallas_call(
            lambda *refs: _kernel(*refs, cfg=cfg),
            out_shape=jax.ShapeDtypeStruct(A_x.shape, A_x.dtype),
            in_specs=[hbm] * 9,
            out_specs=hbm,
            scratch_shapes=[
                pltpu.VMEM((1, 1, D), BF16),
                pltpu.VMEM((1, D), BF16),
                pltpu.VMEM((4, D // 4, GATE), BF16),
                pltpu.VMEM((D, 6 * D - GATE), BF16),
                pltpu.VMEM((4, D // 4, HQ * DH), BF16),
                pltpu.VMEM((window // STEP, 4, 2, STEP, DH), BF16),
                pltpu.VMEM((window // STEP, 4, 2, STEP, DH), BF16),
                pltpu.VMEM((4, D // 4, HQ * DH), BF16),
                pltpu.VMEM((4, D // 4, F), BF16),
                pltpu.VMEM((D, F), BF16),
                pltpu.VMEM((HKV, ROWS, DH), F32),
                pltpu.VMEM((HKV, ROWS, window), F32),
                pltpu.VMEM((HKV, ROWS, 128), F32),
                pltpu.VMEM((ROWS, HQ * DH), F32),
                pltpu.VMEM((6, ROWS, D), F32),
                pltpu.VMEM((512, 128), F32),
                pltpu.VMEM((2, ROWS, 512), F32),
                pltpu.VMEM((1, 1, D), BF16),
                pltpu.SemaphoreType.DMA((S_GATE + len(cfg['gate']) - 1,)),
            ],
            compiler_params=pltpu.CompilerParams(
                vmem_limit_bytes=100 * 2**20,
                disable_semaphore_checks=True,
                disable_bounds_checks=True,
            ),
            interpret=interpret,
            name="adaln_decode",
        )(A_x, c, w_mod.reshape(4, D // 4, -1), A_wq.reshape(4, D // 4, -1), A_k_cache.reshape(2, 4, keys, DH), A_v_cache.reshape(2, 4, keys, DH), A_wo.T.reshape(4, D // 4, -1), B_w3.reshape(4, D // 4, -1), B_w4.T)
    return run


pallas_adaLN_cond__sliding_block_cached__mixer_s_mlp__decode_kernel = build()
```

```python
import jax
import jax.numpy as jnp
from jax import lax
from jax.experimental import pallas as pl
from jax.experimental.pallas import tpu as pltpu

D, F = 448, 1792
HQ, HKV, DH = 16, 8, 256
EPS = 1e-5
ROWS = 8
STEP = 32
ROUNDS = 8
AHEAD = 26
TILE_ROWS = D // 8
GATE = 2304
BF16, F32 = jnp.bfloat16, jnp.float32
CFG = dict(skew=60, heads=(0, 1, 2, 3, 4, 5, 6, 7), z=2, w4=((64, 128), (192, 128), (320, 128), (0, 64)),
           gate=(0, 12, 18, 22, 25, 28), at={}, early=12, hold=4, mid=16, order=((0, 2), (1,), (3,)))

S_X, S_C, S_WM, S_WQ, S_WO, S_W3, S_K, S_V, S_W4, S_GATE = 0, 1, 2, 3, 4, 5, 6, 14, 22, 26


def _layernorm(x):
    d = x - jnp.sum(x, axis=-1, keepdims=True) * (1.0 / D)
    return d * lax.rsqrt(jnp.sum(d * d, axis=-1, keepdims=True) * (1.0 / D) + EPS)


def _dot(a, b):
    return lax.dot_general(a, b, (((1,), (0,)), ((), ())), preferred_element_type=F32)


def _dot_t(a, b):
    return lax.dot_general(a, b, (((1,), (1,)), ((), ())), preferred_element_type=F32)


def _ds(start, size):
    return pl.ds(start if isinstance(start, int) else pl.multiple_of(start, size), size)


def _lanes(x, op):
    out = x[:, :128]
    for t in range(128, x.shape[1], 128):
        out = op(out, x[:, t:t + 128])
    return out


def _merge(a, b):
    order = sorted([((i + 0.5) / len(a), 0, i) for i in range(len(a))] + [((i + 0.5) / len(b), 1, i) for i in range(len(b))])
    return [(a, b)[which][i] for _, which, i in order]


def _kernel(x_hbm, c_hbm, wm_hbm, wq_hbm, k_hbm, v_hbm, wo_hbm, w3_hbm, w4_hbm, out_hbm,
            x_ref, c_ref, wm_ref, gate_ref, wq_ref, k_ref, v_ref, wo_ref, w3_ref, w4_ref,
            q_ref, s_ref, max_ref, acc_ref, ctx_ref, mod_ref, cond_ref, last_ref, out_ref, sems, *, cfg):
    steps = k_ref.shape[0]
    block = 2 * ROUNDS * STEP
    blocks = steps // ROUNDS

    def cache(hbm, ref, sem):
        def copy(b, i):
            b, i = b + i // (ROUNDS * HKV), i % (ROUNDS * HKV)
            j, h = b * ROUNDS + i // HKV, cfg['heads'][i % HKV]
            rows = _ds(((j + cfg['skew'] * h) & (steps - 1)) * STEP, STEP)
            return pltpu.make_async_copy(hbm.at[h, pl.ds(hbm.shape[1] - 2, 2), rows], ref.at[j, h], sems.at[sem + b])
        return copy

    def streams(hbm, ref, sem, n, cuts):
        spots = [(slice(None), pl.ds(row, 8), pl.ds(128 * lo, 128 * (hi - lo)))
                 for row in range(0, D // n, 8) for lo, hi in zip(cuts[:-1], cuts[1:])]
        return [pltpu.make_async_copy(hbm.at[at], ref.at[at], sems.at[sem]) for at in spots]

    keys, values = cache(k_hbm, k_ref, S_K), cache(v_hbm, v_ref, S_V)
    wq, wo = streams(wq_hbm, wq_ref, S_WQ, 4, range(0, 33, 4)), streams(wo_hbm, wo_ref, S_WO, 4, range(0, 33, 4))
    wm = streams(wm_hbm, wm_ref, S_WM, 4, (0, 5, 9, 14, 18))
    w3 = streams(w3_hbm, w3_ref, S_W3, 4, (0, 4, 8, 11, 14))
    w4 = [[pltpu.make_async_copy(w4_hbm.at[pl.ds(row, 8)], w4_ref.at[pl.ds(row, 8)], sems.at[S_W4 + i])
           for row in range(r0, r0 + n, 8)] for i, (r0, n) in enumerate(cfg['w4'])]
    groups = list(zip(cfg['gate'][:-1], cfg['gate'][1:]))
    gate = [pltpu.make_async_copy(wm_hbm.at[j // 7, pl.ds(j % 7 * 16, 16), pl.ds(GATE, 6 * D - GATE)], gate_ref.at[pl.ds(16 * j, 16)],
                                  sems.at[S_GATE + i]) for i, (lo, hi) in enumerate(groups) for j in range(lo, hi)]
    small = [pltpu.make_async_copy(c_hbm, c_ref, sems.at[S_C]), pltpu.make_async_copy(x_hbm, x_ref, sems.at[S_X])]

    def landed(ref, sem):
        pltpu.make_async_copy(ref, ref, sems.at[sem]).wait()

    even = (lax.broadcasted_iota(jnp.int32, (ROWS, DH), 0) & 1) == 0
    live = {}

    def condition():
        for copy in small:
            copy.wait()
        landed(wm_ref, S_WM)
        c = jnp.broadcast_to(c_ref[...].astype(F32), (ROWS, D))
        c = (c * jax.nn.sigmoid(c)).astype(BF16)
        mod = _dot(c, wm_ref[...].reshape(D, GATE))
        for g in range(5):
            mod_ref[g] = mod[:, g * D:(g + 1) * D]
        mod_ref[5, :, :GATE - 5 * D] = mod[:, 5 * D:]
        wide = jnp.concatenate([c.astype(F32), jnp.zeros((ROWS, 512 - D), F32)], axis=1)
        cond_ref[...] = jnp.concatenate([wide] * (128 // ROWS), axis=0).T

    def queries():
        landed(wq_ref, S_WQ)
        x = jnp.broadcast_to(x_ref[0].astype(F32), (ROWS, D))
        h = (_layernorm(x) * (1.0 + mod_ref[1]) + mod_ref[0]).astype(BF16)
        q = _dot(h, wq_ref[...].reshape(D, HQ * DH)) * DH ** -0.5
        for i in range(HKV):
            q_ref[i] = jnp.where(even, q[:, 2 * i * DH:(2 * i + 1) * DH], q[:, (2 * i + 1) * DH:(2 * i + 2) * DH])
            max_ref[i] = jnp.full((ROWS, 128), -jnp.inf, F32)

    def scores(b):
        rounds = pl.ds(b * ROUNDS, ROUNDS)
        landed(k_ref.at[rounds], S_K + b)
        for h in range(HKV):
            s = _dot_t(q_ref[h].astype(BF16), k_ref[rounds, h].reshape(block, DH))
            s_ref[h, :, _ds(b * block, block)] = s
            max_ref[h] = jnp.maximum(max_ref[h], _lanes(s, jnp.maximum))

    def softmax():
        def body(h, carry):
            p = jnp.exp(s_ref[h] - jnp.max(max_ref[h], axis=-1, keepdims=True))
            s_ref[h] = p
            max_ref[h] = jnp.broadcast_to(jnp.sum(_lanes(p, jnp.add), axis=-1, keepdims=True), (ROWS, 128))
            acc_ref[h] = jnp.zeros((ROWS, DH), F32)
            return carry
        lax.fori_loop(0, HKV, body, None)

    def context(b, last=False):
        rounds = pl.ds(b * ROUNDS, ROUNDS)
        landed(v_ref.at[rounds], S_V + b)
        for h in range(HKV):
            o = acc_ref[h] + _dot(s_ref[h, :, _ds(b * block, block)].astype(BF16), v_ref[rounds, h].reshape(block, DH))
            if last:
                o = o / jnp.concatenate([max_ref[h]] * 2, axis=1)
                ctx_ref[:, 2 * h * DH:(2 * h + 2) * DH] = jnp.concatenate([jnp.where(even, o, 0.0), jnp.where(even, 0.0, o)], axis=1)
            else:
                acc_ref[h] = o

    def project(part):
        if part == 0:
            landed(wo_ref, S_WO)

        def body(i, attn):
            cols = _ds(i * 1024, 1024)
            return attn + _dot_t(ctx_ref[:, cols].astype(BF16), wo_ref[:, :, cols].reshape(D, 1024))
        live['attn'] = lax.fori_loop(2 * part, 2 * part + 2, body, live['attn'] if part else jnp.zeros((ROWS, D), F32))

    def residual():
        attn = live['attn'] + pltpu.roll(live['attn'], 1, 0)
        x = jnp.broadcast_to(x_ref[0].astype(F32), (ROWS, D)) + mod_ref[2] * attn
        h = _layernorm(x) * (1.0 + mod_ref[4]) + mod_ref[3]
        live['normed'] = _layernorm(h).astype(BF16)
        for i, v in enumerate((x, h)):
            last_ref[i] = jnp.concatenate([v[:, 64:], v[:, :128]], axis=1)

    early, hold, mid = cfg['early'], cfg['hold'], cfg['mid']
    outer = _merge(w4[0], w4[2])
    back = _merge(w3[early:], outer[:mid]) + outer[mid:] + _merge(w4[1], w4[3][:8 - hold]) + w4[3][8 - hold:]
    if cfg['z']:
        front = wm + _merge(wq, wo) if cfg['z'] == 1 else _merge(wm, _merge(wq, wo))
        back = w3[:early] + back
        at = dict(cond=10, q=31, c=29, p0=36, p1=44, r=52)
    else:
        front = _merge(wm, wq)
        back = _merge(wo, w3[:early]) + back
        at = dict(cond=29, q=40, c=32, p0=89, p1=96, r=103)
    at.update(cfg['at'])
    spare = len(gate) - AHEAD
    back, gate = back + gate[:spare], gate[spare:]
    n = ROUNDS * HKV * blocks

    def item(i):
        i -= len(front)
        return front[i] if i < 0 else keys(0, i) if i < n else values(0, i - n) if i < 2 * n else back[i - 2 * n]

    start, stop = len(front) // 2, (len(front) + 2 * n + len(back)) // 2

    def pairs(lo, hi, work):
        for i in range(lo, hi):
            if i in work:
                work.pop(i)()
            (item(2 * (i + AHEAD)) if i + AHEAD < stop else gate[i + AHEAD - stop]).start(priority=1)
            item(2 * i + 1).start(priority=0)
        for i in sorted(work):
            work[i]()

    def loop(copy, work):
        def body(b, carry):
            work(b - 2)
            for i in range(0, ROUNDS * HKV, 2):
                copy(b, i + 2 * AHEAD).start(priority=1)
                copy(b, i + 1).start(priority=0)
            return carry
        lax.fori_loop(2, blocks - 1, body, None)

    for i in range(AHEAD):
        item(2 * i).start(priority=1)
    for copy in small:
        copy.start(priority=0)
    pairs(0, start + 64, {start + at['cond']: condition, start + at['q']: queries})
    loop(keys, scores)
    at_v, at_end = start + n // 2, start + n
    pairs(at_v - 32, at_v + 64, {at_v - 32: lambda: scores(blocks - 3), at_v: lambda: scores(blocks - 2),
                                 at_v + 32: lambda: scores(blocks - 1), at_v + 48: softmax})
    loop(values, context)
    pairs(at_end - 32, stop, {at_end - 32: lambda: context(blocks - 3), at_end: lambda: context(blocks - 2),
                              at_end + at['c']: lambda: context(blocks - 1, True), at_end + at['p0']: lambda: project(0),
                              at_end + at['p1']: lambda: project(1), at_end + at['r']: residual})

    landed(w3_ref, S_W3)
    hidden = jax.nn.gelu(_dot(live['normed'], w3_ref[...].reshape(D, F)), approximate=True).astype(BF16)
    y = [None] * 4
    acc = [None] * 3
    for batch in cfg.get('order', ((0, 2), (1, 3))) + tuple((4 + i,) for i in range(len(groups))):
        for i in batch:
            if i < 4:
                landed(w4_ref.at[pl.ds(*cfg['w4'][i])], S_W4 + i)
            else:
                lo, hi = groups[i - 4]
                landed(gate_ref.at[pl.ds(16 * lo, 16 * (hi - lo))], S_GATE + i - 4)
        for i in batch:
            if i < 4:
                r0, n = cfg['w4'][i]
                y[i] = last_ref[1, :, 128 * i:128 * i + n] + (0.0 if cfg.get('dry') == 2 else _dot_t(hidden, w4_ref[r0:r0 + n, :]))
                continue
            for j in range(*groups[i - 4]):
                for t in range(3):
                    w = gate_ref[16 * j:16 * j + 16, 128 * t:128 * t + 128].astype(F32) * cond_ref[16 * j:16 * j + 16, :]
                    w = w[:ROWS] + w[ROWS:]
                    acc[t] = w if acc[t] is None else acc[t] + w
    head = last_ref[0, :, 384:448] + mod_ref[5, :, :64] * y[3]
    turned = [jnp.concatenate([head, jnp.zeros_like(head)], axis=1)]
    for t in range(3):
        for step in (4, 2, 1):
            acc[t] = acc[t] + pltpu.roll(acc[t], step, 0)
        turned.append(pltpu.roll(last_ref[0, :, 128 * t:128 * t + 128] + acc[t] * y[t], 0 if cfg.get('norot') else 64, 1))
    low = lax.broadcasted_iota(jnp.int32, (ROWS, 128), 1) < 64
    tiles = [jnp.where(low, turned[t], turned[t + 1]) for t in range(3)] + [turned[3][:, :64]]
    out_ref[0] = jnp.concatenate(tiles, axis=1)[:1].astype(BF16)
    store = pltpu.make_async_copy(out_ref, out_hbm, sems.at[S_X])
    store.start()
    store.wait()


def build(interpret=False, **changes):
    cfg = dict(CFG, **changes)

    @jax.jit
    def run(A_x, A_k_cache, A_v_cache, A_wq, A_wo, B_x, B_w1, B_w2, B_w3, B_w4, c, w_mod):
        keys = A_k_cache.shape[2]
        window = min(4096, max(256, keys // 4))
        assert A_x.shape == (1, 1, D) and A_k_cache.shape == (1, HKV, keys, DH) and window == 4096
        hbm = pl.BlockSpec(memory_space=pltpu.HBM)
        return pl.pallas_call(
            lambda *refs: _kernel(*refs, cfg=cfg),
            out_shape=jax.ShapeDtypeStruct(A_x.shape, A_x.dtype),
            in_specs=[hbm] * 9,
            out_specs=hbm,
            scratch_shapes=[
                pltpu.VMEM((1, 1, D), BF16),
                pltpu.VMEM((1, D), BF16),
                pltpu.VMEM((4, D // 4, GATE), BF16),
                pltpu.VMEM((D, 6 * D - GATE), BF16),
                pltpu.VMEM((4, D // 4, HQ * DH), BF16),
                pltpu.VMEM((window // STEP // 2, HKV, 2, STEP, DH), BF16),
                pltpu.VMEM((window // STEP // 2, HKV, 2, STEP, DH), BF16),
                pltpu.VMEM((4, D // 4, HQ * DH), BF16),
                pltpu.VMEM((4, D // 4, F), BF16),
                pltpu.VMEM((D, F), BF16),
                pltpu.VMEM((HKV, ROWS, DH), F32),
                pltpu.VMEM((HKV, ROWS, window), F32),
                pltpu.VMEM((HKV, ROWS, 128), F32),
                pltpu.VMEM((HKV, ROWS, DH), F32),
                pltpu.VMEM((ROWS, HQ * DH), F32),
                pltpu.VMEM((6, ROWS, D), F32),
                pltpu.VMEM((512, 128), F32),
                pltpu.VMEM((2, ROWS, 512), F32),
                pltpu.VMEM((1, 1, D), BF16),
                pltpu.SemaphoreType.DMA((S_GATE + len(cfg['gate']) - 1,)),
            ],
            compiler_params=pltpu.CompilerParams(
                vmem_limit_bytes=100 * 2**20,
                disable_semaphore_checks=True,
                disable_bounds_checks=True,
            ),
            interpret=interpret,
            name="adaln_decode",
        )(A_x, c, w_mod.reshape(4, D // 4, -1), A_wq.reshape(4, D // 4, -1), A_k_cache.reshape(HKV, -1, window // 2, DH), A_v_cache.reshape(HKV, -1, window // 2, DH), A_wo.T.reshape(4, D // 4, -1), B_w3.reshape(4, D // 4, -1), B_w4.T)
    return run


pallas_adaLN_cond__sliding_block_cached__mixer_s_mlp__decode_kernel = build()
```

```python
import jax
import jax.numpy as jnp
from jax import lax
from jax.experimental import pallas as pl
from jax.experimental.pallas import tpu as pltpu

D, F = 448, 1792
HQ, HKV, DH = 16, 8, 256
EPS = 1e-5
BF16, F32 = jnp.bfloat16, jnp.float32
ROWS = 8
AHEAD = 26

STEP = 32
HEADS = (7, 3, 4, 6, 2, 1, 0, 5)
FIRST = (48, 6, 56, 61, 48, 54, 40, 60)
ROUNDS = 8

GATE = 2304
OUT_BLOCKS = ((64, 128), (192, 128), (320, 128), (0, 64))
GATE_BLOCKS = ((0, 192), (192, 96), (288, 64), (352, 48), (400, 48))

S_X, S_C, S_WM, S_WQ, S_WO, S_W3, S_K, S_V, S_W4, S_GATE = 0, 1, 2, 3, 4, 5, 6, 14, 22, 26


def _layernorm(x):
    d = x - jnp.sum(x, axis=-1, keepdims=True) * (1.0 / D)
    return d * lax.rsqrt(jnp.sum(d * d, axis=-1, keepdims=True) * (1.0 / D) + EPS)


def _dot(a, b):
    return lax.dot_general(a, b, (((1,), (0,)), ((), ())), preferred_element_type=F32)


def _dot_t(a, b):
    return lax.dot_general(a, b, (((1,), (1,)), ((), ())), preferred_element_type=F32)


def _ds(start, size):
    return pl.ds(start if isinstance(start, int) else pl.multiple_of(start, size), size)


def _fold(op, x):
    out = x[:, :128]
    for t in range(128, x.shape[1], 128):
        out = op(out, x[:, t:t + 128])
    return out


def _merge(*lists):
    order = sorted(((i + 0.5) / len(items), k, i) for k, items in enumerate(lists) for i in range(len(items)))
    return [lists[k][i] for _, k, i in order]


def _kernel(x_hbm, c_hbm, wm_hbm, wq_hbm, k_hbm, v_hbm, wo_hbm, w3_hbm, w4_hbm, out_hbm,
            x_ref, c_ref, wm_ref, gate_ref, wq_ref, k_ref, v_ref, wo_ref, w3_ref, w4_ref,
            cond_ref, mod_ref, q_ref, s_ref, stat_ref, acc_ref, ctx_ref, mlp_ref, out_ref, sems):
    steps = k_ref.shape[0]
    blocks, per_block = steps // ROUNDS, ROUNDS * HKV
    block_keys = 2 * ROUNDS * STEP

    def cache(hbm, ref, sem):
        def copy(b, i):
            b, i = b + i // per_block, i % per_block
            j, h = b * ROUNDS + i // HKV, HEADS[i % HKV]
            rows = _ds(((j + FIRST[h]) & (steps - 1)) * STEP, STEP)
            return pltpu.make_async_copy(hbm.at[h, pl.ds(hbm.shape[1] - 2, 2), rows], ref.at[j, h], sems.at[sem + b])
        return copy

    def weight(hbm, ref, sem, cuts):
        spots = [(slice(None), pl.ds(row, 8), pl.ds(128 * lo, 128 * (hi - lo)))
                 for row in range(0, ref.shape[1], 8) for lo, hi in zip(cuts[:-1], cuts[1:])]
        return [pltpu.make_async_copy(hbm.at[at], ref.at[at], sems.at[sem]) for at in spots]

    def two_ways(copies):
        return _merge(copies[:len(copies) // 2], copies[len(copies) // 2:])

    keys, values = cache(k_hbm, k_ref, S_K), cache(v_hbm, v_ref, S_V)
    inputs = [pltpu.make_async_copy(c_hbm, c_ref, sems.at[S_C]), pltpu.make_async_copy(x_hbm, x_ref, sems.at[S_X])]
    wm = weight(wm_hbm, wm_ref, S_WM, (0, 9, 18))
    wq = two_ways(weight(wq_hbm, wq_ref, S_WQ, (0, 8, 16, 24, 32)))
    wo = two_ways(weight(wo_hbm, wo_ref, S_WO, (0, 8, 16, 24, 32)))
    w3 = weight(w3_hbm, w3_ref, S_W3, (0, 4, 8, 11, 14))
    w4 = [[pltpu.make_async_copy(w4_hbm.at[pl.ds(row, 8)], w4_ref.at[pl.ds(row, 8)], sems.at[S_W4 + i])
           for row in range(lo, lo + n, 8)] for i, (lo, n) in enumerate(OUT_BLOCKS)]
    gate = [pltpu.make_async_copy(wm_hbm.at[row // (D // 2), pl.ds(row % (D // 2), 16), pl.ds(GATE, 6 * D - GATE)],
                                  gate_ref.at[pl.ds(row, 16)], sems.at[S_GATE + i])
            for i, (lo, n) in enumerate(GATE_BLOCKS) for row in range(lo, lo + n, 16)]

    def landed(ref, sem):
        pltpu.make_async_copy(ref, ref, sems.at[sem]).wait()

    even = (lax.broadcasted_iota(jnp.int32, (ROWS, DH), 0) & 1) == 0
    live = {"attn": jnp.zeros((ROWS, D), F32)}

    def condition():
        for copy in inputs:
            copy.wait()
        landed(wm_ref, S_WM)
        c = jnp.broadcast_to(c_ref[...].astype(F32), (ROWS, D))
        c = (c * jax.nn.sigmoid(c)).astype(BF16)
        mod = _dot(c, wm_ref[...].reshape(D, GATE))
        for g in range(5):
            mod_ref[g] = mod[:, g * D:(g + 1) * D]
        mod_ref[5, :, :GATE - 5 * D] = mod[:, 5 * D:]
        wide = jnp.concatenate([c.astype(F32), jnp.zeros((ROWS, 512 - D), F32)], axis=1)
        cond_ref[...] = jnp.concatenate([wide] * (128 // ROWS), axis=0).T

    def queries():
        landed(wq_ref, S_WQ)
        x = jnp.broadcast_to(x_ref[0].astype(F32), (ROWS, D))
        h = (_layernorm(x) * (1.0 + mod_ref[1]) + mod_ref[0]).astype(BF16)
        q = _dot(h, wq_ref[...].reshape(D, HQ * DH)) * DH ** -0.5
        for i in range(HKV):
            q_ref[i] = jnp.where(even, q[:, 2 * i * DH:(2 * i + 1) * DH], q[:, (2 * i + 1) * DH:(2 * i + 2) * DH])
            stat_ref[i] = jnp.full((ROWS, 128), -jnp.inf, F32)

    def scores(b):
        rounds = pl.ds(b * ROUNDS, ROUNDS)
        landed(k_ref.at[rounds], S_K + b)
        for h in range(HKV):
            s = _dot_t(q_ref[h].astype(BF16), k_ref[rounds, h].reshape(block_keys, DH))
            s_ref[h, :, _ds(b * block_keys, block_keys)] = s
            stat_ref[h] = jnp.maximum(stat_ref[h], _fold(jnp.maximum, s))

    def softmax():
        def body(h, carry):
            p = jnp.exp(s_ref[h] - jnp.max(stat_ref[h], axis=-1, keepdims=True))
            s_ref[h] = p
            stat_ref[h] = jnp.broadcast_to(jnp.sum(_fold(jnp.add, p), axis=-1, keepdims=True), (ROWS, 128))
            acc_ref[h] = jnp.zeros((ROWS, DH), F32)
            return carry
        lax.fori_loop(0, HKV, body, None)

    def context(b, last=False):
        rounds = pl.ds(b * ROUNDS, ROUNDS)
        landed(v_ref.at[rounds], S_V + b)
        for h in range(HKV):
            p = s_ref[h, :, _ds(b * block_keys, block_keys)].astype(BF16)
            o = acc_ref[h] + _dot(p, v_ref[rounds, h].reshape(block_keys, DH))
            if last:
                o = o / jnp.concatenate([stat_ref[h]] * (DH // 128), axis=1)
                ctx_ref[:, 2 * h * DH:(2 * h + 2) * DH] = jnp.concatenate(
                    [jnp.where(even, o, 0.0), jnp.where(even, 0.0, o)], axis=1)
            else:
                acc_ref[h] = o

    def project(part):
        if part == 0:
            landed(wo_ref, S_WO)

        def body(i, attn):
            cols = _ds(i * 1024, 1024)
            return attn + _dot_t(ctx_ref[:, cols].astype(BF16), wo_ref[:, :, cols].reshape(D, 1024))
        live["attn"] = lax.fori_loop(2 * part, 2 * part + 2, body, live["attn"])

    def residual():
        attn = live["attn"] + pltpu.roll(live["attn"], 1, 0)
        x = jnp.broadcast_to(x_ref[0].astype(F32), (ROWS, D)) + mod_ref[2] * attn
        h = _layernorm(x) * (1.0 + mod_ref[4]) + mod_ref[3]
        live["normed"] = _layernorm(h).astype(BF16)
        for i, v in enumerate((x, h)):
            mlp_ref[i] = jnp.concatenate([v[:, 64:], v[:, :128]], axis=1)

    outer = _merge(w4[0], w4[2])
    front = _merge(wm, _merge(wq, wo))
    back = _merge(w3, outer[:16]) + outer[16:] + w4[1] + w4[3] + gate
    back, tail = back[:-AHEAD], back[-AHEAD:]
    n = blocks * per_block

    def item(i):
        i -= len(front)
        return front[i] if i < 0 else keys(0, i) if i < n else values(0, i - n) if i < 2 * n else back[i - 2 * n]

    at_k = len(front) // 2
    at_v, at_back = at_k + n // 2, at_k + n
    end, block = at_back + len(back) // 2, per_block // 2

    def pairs(lo, hi, work):
        for i in range(lo, hi):
            if i in work:
                work[i]()
            (item(2 * (i + AHEAD)) if i + AHEAD < end else tail[i + AHEAD - end]).start(priority=1)
            item(2 * i + 1).start(priority=0)

    def loop(copy, work):
        def body(b, carry):
            work(b - 2)
            for i in range(0, per_block, 2):
                copy(b, i + 2 * AHEAD).start(priority=1)
                copy(b, i + 1).start(priority=0)
            return carry
        lax.fori_loop(2, blocks - 1, body, None)

    for i in range(AHEAD):
        item(2 * i).start(priority=1)
    for copy in inputs:
        copy.start(priority=0)
    pairs(0, at_k + 2 * block, {at_k + 29: condition, at_k + 40: queries})
    loop(keys, scores)
    pairs(at_v - block, at_v + 2 * block,
          {at_v - block: lambda: scores(blocks - 3), at_v: lambda: scores(blocks - 2),
           at_v + block: lambda: scores(blocks - 1), at_v + 48: softmax})
    loop(values, context)
    pairs(at_back - block, end,
          {at_back - block: lambda: context(blocks - 3), at_back: lambda: context(blocks - 2),
           at_back + 29: lambda: context(blocks - 1, last=True), at_back + 36: lambda: project(0),
           at_back + 44: lambda: project(1), at_back + 52: residual})

    landed(w3_ref, S_W3)
    hidden = jax.nn.gelu(_dot(live["normed"], w3_ref[...].reshape(D, F)), approximate=True).astype(BF16)
    y = {}
    for batch in ((0, 2), (1,), (3,)):
        for i in batch:
            landed(w4_ref.at[pl.ds(*OUT_BLOCKS[i])], S_W4 + i)
        for i in batch:
            lo, width = OUT_BLOCKS[i]
            y[i] = mlp_ref[1, :, 128 * i:128 * i + width] + _dot_t(hidden, w4_ref[lo:lo + width, :])

    sums = [jnp.zeros((ROWS, 128), F32)] * 3
    for i, (lo, rows) in enumerate(GATE_BLOCKS):
        landed(gate_ref.at[pl.ds(lo, rows)], S_GATE + i)
        for row in range(lo, lo + rows, 16):
            for t in range(3):
                w = gate_ref[row:row + 16, 128 * t:128 * t + 128].astype(F32) * cond_ref[row:row + 16, :]
                sums[t] = sums[t] + (w[:ROWS] + w[ROWS:])
    for shift in (4, 2, 1):
        sums = [s + pltpu.roll(s, shift, 0) for s in sums]
    sublane = lax.broadcasted_iota(jnp.int32, (ROWS, 128), 0)
    stack = lambda tiles: jnp.where(sublane < 2, tiles[0], jnp.where(sublane < 4, tiles[1], tiles[2]))
    x = stack([mlp_ref[0, :, 128 * t:128 * t + 128] for t in range(3)])
    turned = pltpu.roll(x + stack(sums) * stack(y), 64, 1)
    head = mlp_ref[0, :, 384:448] + mod_ref[5, :, :64] * y[3]
    turned = [jnp.concatenate([head, jnp.zeros_like(head)], axis=1)[:1], turned[:1], turned[2:3], turned[4:5]]
    low = lax.broadcasted_iota(jnp.int32, (1, 128), 1) < 64
    tiles = [jnp.where(low, turned[t], turned[t + 1]) for t in range(3)] + [turned[3][:, :64]]
    out_ref[0] = jnp.concatenate(tiles, axis=1).astype(BF16)
    store = pltpu.make_async_copy(out_ref, out_hbm, sems.at[S_X])
    store.start()
    store.wait()


@jax.jit
def pallas_adaLN_cond__sliding_block_cached__mixer_s_mlp__decode_kernel(
    A_x: jax.Array,
    A_k_cache: jax.Array,
    A_v_cache: jax.Array,
    A_wq: jax.Array,
    A_wo: jax.Array,
    B_x: jax.Array,
    B_w1: jax.Array,
    B_w2: jax.Array,
    B_w3: jax.Array,
    B_w4: jax.Array,
    c: jax.Array,
    w_mod: jax.Array,
):
    keys = A_k_cache.shape[2]
    window = min(4096, max(256, keys // 4))
    assert A_x.shape == (1, 1, D) and A_k_cache.shape == (1, HKV, keys, DH)
    assert window == 4096 and keys % (window // 2) == 0
    halves = lambda a: a.reshape(HKV, -1, window // 2, DH)
    slabs = lambda w, n: w.reshape(n, D // n, -1)
    steps = window // 2 // STEP
    hbm = pl.BlockSpec(memory_space=pltpu.HBM)
    return pl.pallas_call(
        _kernel,
        out_shape=jax.ShapeDtypeStruct(A_x.shape, A_x.dtype),
        in_specs=[hbm] * 9,
        out_specs=hbm,
        scratch_shapes=[
            pltpu.VMEM((1, 1, D), BF16),
            pltpu.VMEM((1, D), BF16),
            pltpu.VMEM((2, D // 2, GATE), BF16),
            pltpu.VMEM((D, 6 * D - GATE), BF16),
            pltpu.VMEM((2, D // 2, HQ * DH), BF16),
            pltpu.VMEM((steps, HKV, 2, STEP, DH), BF16),
            pltpu.VMEM((steps, HKV, 2, STEP, DH), BF16),
            pltpu.VMEM((2, D // 2, HQ * DH), BF16),
            pltpu.VMEM((4, D // 4, F), BF16),
            pltpu.VMEM((D, F), BF16),
            pltpu.VMEM((512, 128), F32),
            pltpu.VMEM((6, ROWS, D), F32),
            pltpu.VMEM((HKV, ROWS, DH), F32),
            pltpu.VMEM((HKV, ROWS, window), F32),
            pltpu.VMEM((HKV, ROWS, 128), F32),
            pltpu.VMEM((HKV, ROWS, DH), F32),
            pltpu.VMEM((ROWS, HQ * DH), F32),
            pltpu.VMEM((2, ROWS, 512), F32),
            pltpu.VMEM((1, 1, D), BF16),
            pltpu.SemaphoreType.DMA((S_GATE + len(GATE_BLOCKS),)),
        ],
        compiler_params=pltpu.CompilerParams(
            vmem_limit_bytes=100 * 2**20,
            disable_semaphore_checks=True,
        ),
        name="adaln_decode",
    )(A_x, c, slabs(w_mod, 2), slabs(A_wq, 2), halves(A_k_cache), halves(A_v_cache),
      slabs(A_wo.T, 2), slabs(B_w3, 4), B_w4.T)
```

```python
import jax
import jax.numpy as jnp
from jax import lax
from jax.experimental import pallas as pl
from jax.experimental.pallas import tpu as pltpu

D, F = 448, 1792
HQ, HKV, DH = 16, 8, 256
EPS = 1e-5
BF16, F32 = jnp.bfloat16, jnp.float32
ROWS = 8
AHEAD = 26

STEP = 32
HEADS = (4, 1, 6, 3, 0, 5, 2, 7)
FIRST = (63, 60, 55, 52, 46, 44, 38, 36)
ROUNDS = 8

GATE = 2304
OUT_BLOCKS = ((64, 128), (192, 128), (320, 128), (0, 64))
GATE_BLOCKS = ((0, 192), (192, 96), (288, 64), (352, 48), (400, 48))

S_X, S_C, S_WM, S_WQ, S_WO, S_W3, S_K, S_V, S_W4, S_GATE = 0, 1, 2, 3, 4, 5, 6, 14, 22, 26


def _layernorm(x):
    d = x - jnp.sum(x, axis=-1, keepdims=True) * (1.0 / D)
    return d * lax.rsqrt(jnp.sum(d * d, axis=-1, keepdims=True) * (1.0 / D) + EPS)


def _dot(a, b):
    return lax.dot_general(a, b, (((1,), (0,)), ((), ())), preferred_element_type=F32)


def _dot_t(a, b):
    return lax.dot_general(a, b, (((1,), (1,)), ((), ())), preferred_element_type=F32)


def _ds(start, size):
    return pl.ds(start if isinstance(start, int) else pl.multiple_of(start, size), size)


def _fold(op, x):
    out = x[:, :128]
    for t in range(128, x.shape[1], 128):
        out = op(out, x[:, t:t + 128])
    return out


def _merge(*lists):
    order = sorted(((i + 0.5) / len(items), k, i) for k, items in enumerate(lists) for i in range(len(items)))
    return [lists[k][i] for _, k, i in order]


def _kernel(x_hbm, c_hbm, wm_hbm, wq_hbm, k_hbm, v_hbm, wo_hbm, w3_hbm, w4_hbm, out_hbm,
            x_ref, c_ref, wm_ref, gate_ref, wq_ref, k_ref, v_ref, wo_ref, w3_ref, w4_ref,
            cond_ref, mod_ref, q_ref, s_ref, stat_ref, acc_ref, ctx_ref, mlp_ref, out_ref, sems):
    steps = k_ref.shape[0]
    blocks, per_block = steps // ROUNDS, ROUNDS * HKV
    block_keys = 2 * ROUNDS * STEP

    def cache(hbm, ref, sem):
        def copy(b, i):
            b, i = b + i // per_block, i % per_block
            j, h = b * ROUNDS + i // HKV, HEADS[i % HKV]
            rows = _ds(((j + FIRST[h]) & (steps - 1)) * STEP, STEP)
            return pltpu.make_async_copy(hbm.at[h, pl.ds(hbm.shape[1] - 2, 2), rows], ref.at[j, h], sems.at[sem + b])
        return copy

    def weight(hbm, ref, sem, cuts):
        spots = [(slice(None), pl.ds(row, 8), pl.ds(128 * lo, 128 * (hi - lo)))
                 for row in range(0, ref.shape[1], 8) for lo, hi in zip(cuts[:-1], cuts[1:])]
        return [pltpu.make_async_copy(hbm.at[at], ref.at[at], sems.at[sem]) for at in spots]

    def two_ways(copies):
        return _merge(copies[:len(copies) // 2], copies[len(copies) // 2:])

    keys, values = cache(k_hbm, k_ref, S_K), cache(v_hbm, v_ref, S_V)
    inputs = [pltpu.make_async_copy(c_hbm, c_ref, sems.at[S_C]), pltpu.make_async_copy(x_hbm, x_ref, sems.at[S_X])]
    wm = weight(wm_hbm, wm_ref, S_WM, (0, 9, 18))
    wq = two_ways(weight(wq_hbm, wq_ref, S_WQ, (0, 8, 16, 24, 32)))
    wo = two_ways(weight(wo_hbm, wo_ref, S_WO, (0, 8, 16, 24, 32)))
    w3 = weight(w3_hbm, w3_ref, S_W3, (0, 4, 8, 10, 14))
    w4 = [[pltpu.make_async_copy(w4_hbm.at[pl.ds(row, 8)], w4_ref.at[pl.ds(row, 8)], sems.at[S_W4 + i])
           for row in range(lo, lo + n, 8)] for i, (lo, n) in enumerate(OUT_BLOCKS)]
    gate = [pltpu.make_async_copy(wm_hbm.at[row // (D // 2), pl.ds(row % (D // 2), 16), pl.ds(GATE, 6 * D - GATE)],
                                  gate_ref.at[pl.ds(row, 16)], sems.at[S_GATE + i])
            for i, (lo, n) in enumerate(GATE_BLOCKS) for row in range(lo, lo + n, 16)]

    def landed(ref, sem):
        pltpu.make_async_copy(ref, ref, sems.at[sem]).wait()

    even = (lax.broadcasted_iota(jnp.int32, (ROWS, DH), 0) & 1) == 0
    live = {"attn": jnp.zeros((ROWS, D), F32)}

    def condition():
        for copy in inputs:
            copy.wait()
        landed(wm_ref, S_WM)
        c = jnp.broadcast_to(c_ref[...].astype(F32), (ROWS, D))
        c = (c * jax.nn.sigmoid(c)).astype(BF16)
        mod = _dot(c, wm_ref[...].reshape(D, GATE))
        for g in range(5):
            mod_ref[g] = mod[:, g * D:(g + 1) * D]
        mod_ref[5, :, :GATE - 5 * D] = mod[:, 5 * D:]
        wide = jnp.concatenate([c.astype(F32), jnp.zeros((ROWS, 512 - D), F32)], axis=1)
        cond_ref[...] = jnp.concatenate([wide] * (128 // ROWS), axis=0).T

    def queries():
        landed(wq_ref, S_WQ)
        x = jnp.broadcast_to(x_ref[0].astype(F32), (ROWS, D))
        h = (_layernorm(x) * (1.0 + mod_ref[1]) + mod_ref[0]).astype(BF16)
        q = _dot(h, wq_ref[...].reshape(D, HQ * DH)) * DH ** -0.5
        for i in range(HKV):
            q_ref[i] = jnp.where(even, q[:, 2 * i * DH:(2 * i + 1) * DH], q[:, (2 * i + 1) * DH:(2 * i + 2) * DH])
            stat_ref[i] = jnp.full((ROWS, 128), -jnp.inf, F32)

    def scores(b):
        rounds = pl.ds(b * ROUNDS, ROUNDS)
        landed(k_ref.at[rounds], S_K + b)
        for h in range(HKV):
            s = _dot_t(q_ref[h].astype(BF16), k_ref[rounds, h].reshape(block_keys, DH))
            s_ref[h, :, _ds(b * block_keys, block_keys)] = s
            stat_ref[h] = jnp.maximum(stat_ref[h], _fold(jnp.maximum, s))

    def softmax():
        def body(h, carry):
            p = jnp.exp(s_ref[h] - jnp.max(stat_ref[h], axis=-1, keepdims=True))
            s_ref[h] = p
            stat_ref[h] = jnp.broadcast_to(jnp.sum(_fold(jnp.add, p), axis=-1, keepdims=True), (ROWS, 128))
            acc_ref[h] = jnp.zeros((ROWS, DH), F32)
            return carry
        lax.fori_loop(0, HKV, body, None)

    def context(b, last=False):
        rounds = pl.ds(b * ROUNDS, ROUNDS)
        landed(v_ref.at[rounds], S_V + b)
        for h in range(HKV):
            p = s_ref[h, :, _ds(b * block_keys, block_keys)].astype(BF16)
            o = acc_ref[h] + _dot(p, v_ref[rounds, h].reshape(block_keys, DH))
            if last:
                o = o / jnp.concatenate([stat_ref[h]] * (DH // 128), axis=1)
                ctx_ref[:, 2 * h * DH:(2 * h + 2) * DH] = jnp.concatenate(
                    [jnp.where(even, o, 0.0), jnp.where(even, 0.0, o)], axis=1)
            else:
                acc_ref[h] = o

    def project(part):
        if part == 0:
            landed(wo_ref, S_WO)

        def body(i, attn):
            cols = _ds(i * 1024, 1024)
            return attn + _dot_t(ctx_ref[:, cols].astype(BF16), wo_ref[:, :, cols].reshape(D, 1024))
        live["attn"] = lax.fori_loop(2 * part, 2 * part + 2, body, live["attn"])

    def residual():
        attn = live["attn"] + pltpu.roll(live["attn"], 1, 0)
        x = jnp.broadcast_to(x_ref[0].astype(F32), (ROWS, D)) + mod_ref[2] * attn
        h = _layernorm(x) * (1.0 + mod_ref[4]) + mod_ref[3]
        live["normed"] = _layernorm(h).astype(BF16)
        for i, v in enumerate((x, h)):
            mlp_ref[i] = jnp.concatenate([v[:, 64:], v[:, :128]], axis=1)

    outer = _merge(w4[0], w4[2])
    front = _merge(wm, _merge(wq, wo))
    back = _merge(w3, outer[:20]) + outer[20:] + w4[1] + w4[3] + gate
    back, tail = back[:-AHEAD], back[-AHEAD:]
    n = blocks * per_block

    def item(i):
        i -= len(front)
        return front[i] if i < 0 else keys(0, i) if i < n else values(0, i - n) if i < 2 * n else back[i - 2 * n]

    at_k = len(front) // 2
    at_v, at_back = at_k + n // 2, at_k + n
    end, block = at_back + len(back) // 2, per_block // 2

    def pairs(lo, hi, work):
        for i in range(lo, hi):
            if i in work:
                work[i]()
            (item(2 * (i + AHEAD)) if i + AHEAD < end else tail[i + AHEAD - end]).start(priority=1)
            item(2 * i + 1).start(priority=0)

    def loop(copy, work):
        def body(b, carry):
            work(b - 2)
            for i in range(0, per_block, 2):
                copy(b, i + 2 * AHEAD).start(priority=1)
                copy(b, i + 1).start(priority=0)
            return carry
        lax.fori_loop(2, blocks - 1, body, None)

    item(0).start(priority=1)
    item(1).start(priority=0)
    for i in range(1, AHEAD + 1):
        item(2 * i).start(priority=1)
    for copy in inputs:
        copy.start(priority=0)
    pairs(1, at_k + 2 * block, {at_k + 29: condition, at_k + 40: queries})
    loop(keys, scores)
    pairs(at_v - block, at_v + 2 * block,
          {at_v - block: lambda: scores(blocks - 3), at_v: lambda: scores(blocks - 2),
           at_v + block: lambda: scores(blocks - 1), at_v + 48: softmax})
    loop(values, context)
    pairs(at_back - block, end,
          {at_back - block: lambda: context(blocks - 3), at_back: lambda: context(blocks - 2),
           at_back + 29: lambda: context(blocks - 1, last=True), at_back + 36: lambda: project(0),
           at_back + 44: lambda: project(1), at_back + 52: residual})

    landed(w3_ref, S_W3)
    hidden = jax.nn.gelu(_dot(live["normed"], w3_ref[...].reshape(D, F)), approximate=True).astype(BF16)
    y = {}
    for batch in ((0, 2), (1,), (3,)):
        for i in batch:
            landed(w4_ref.at[pl.ds(*OUT_BLOCKS[i])], S_W4 + i)
        for i in batch:
            lo, width = OUT_BLOCKS[i]
            y[i] = mlp_ref[1, :, 128 * i:128 * i + width] + _dot_t(hidden, w4_ref[lo:lo + width, :])

    sums = [jnp.zeros((ROWS, 128), F32)] * 3
    for i, (lo, rows) in enumerate(GATE_BLOCKS):
        landed(gate_ref.at[pl.ds(lo, rows)], S_GATE + i)
        for row in range(lo, lo + rows, 16):
            for t in range(3):
                w = gate_ref[row:row + 16, 128 * t:128 * t + 128].astype(F32) * cond_ref[row:row + 16, :]
                sums[t] = sums[t] + (w[:ROWS] + w[ROWS:])
    for shift in (4, 2, 1):
        sums = [s + pltpu.roll(s, shift, 0) for s in sums]
    sublane = lax.broadcasted_iota(jnp.int32, (ROWS, 128), 0)
    stack = lambda tiles: jnp.where(sublane < 2, tiles[0], jnp.where(sublane < 4, tiles[1], tiles[2]))
    x = stack([mlp_ref[0, :, 128 * t:128 * t + 128] for t in range(3)])
    turned = pltpu.roll(x + stack(sums) * stack(y), 64, 1)
    head = mlp_ref[0, :, 384:448] + mod_ref[5, :, :64] * y[3]
    turned = [jnp.concatenate([head, jnp.zeros_like(head)], axis=1)[:1], turned[:1], turned[2:3], turned[4:5]]
    low = lax.broadcasted_iota(jnp.int32, (1, 128), 1) < 64
    tiles = [jnp.where(low, turned[t], turned[t + 1]) for t in range(3)] + [turned[3][:, :64]]
    out_ref[0] = jnp.concatenate(tiles, axis=1).astype(BF16)
    store = pltpu.make_async_copy(out_ref, out_hbm, sems.at[S_X])
    store.start()
    store.wait()


@jax.jit
def pallas_adaLN_cond__sliding_block_cached__mixer_s_mlp__decode_kernel(
    A_x: jax.Array,
    A_k_cache: jax.Array,
    A_v_cache: jax.Array,
    A_wq: jax.Array,
    A_wo: jax.Array,
    B_x: jax.Array,
    B_w1: jax.Array,
    B_w2: jax.Array,
    B_w3: jax.Array,
    B_w4: jax.Array,
    c: jax.Array,
    w_mod: jax.Array,
):
    keys = A_k_cache.shape[2]
    window = min(4096, max(256, keys // 4))
    assert A_x.shape == (1, 1, D) and A_k_cache.shape == (1, HKV, keys, DH)
    assert window == 4096 and keys % (window // 2) == 0
    halves = lambda a: a.reshape(HKV, -1, window // 2, DH)
    slabs = lambda w, n: w.reshape(n, D // n, -1)
    steps = window // 2 // STEP
    hbm = pl.BlockSpec(memory_space=pltpu.HBM)
    return pl.pallas_call(
        _kernel,
        out_shape=jax.ShapeDtypeStruct(A_x.shape, A_x.dtype),
        in_specs=[hbm] * 9,
        out_specs=hbm,
        scratch_shapes=[
            pltpu.VMEM((1, 1, D), BF16),
            pltpu.VMEM((1, D), BF16),
            pltpu.VMEM((2, D // 2, GATE), BF16),
            pltpu.VMEM((D, 6 * D - GATE), BF16),
            pltpu.VMEM((2, D // 2, HQ * DH), BF16),
            pltpu.VMEM((steps, HKV, 2, STEP, DH), BF16),
            pltpu.VMEM((steps, HKV, 2, STEP, DH), BF16),
            pltpu.VMEM((2, D // 2, HQ * DH), BF16),
            pltpu.VMEM((4, D // 4, F), BF16),
            pltpu.VMEM((D, F), BF16),
            pltpu.VMEM((512, 128), F32),
            pltpu.VMEM((6, ROWS, D), F32),
            pltpu.VMEM((HKV, ROWS, DH), F32),
            pltpu.VMEM((HKV, ROWS, window), F32),
            pltpu.VMEM((HKV, ROWS, 128), F32),
            pltpu.VMEM((HKV, ROWS, DH), F32),
            pltpu.VMEM((ROWS, HQ * DH), F32),
            pltpu.VMEM((2, ROWS, 512), F32),
            pltpu.VMEM((1, 1, D), BF16),
            pltpu.SemaphoreType.DMA((S_GATE + len(GATE_BLOCKS),)),
        ],
        compiler_params=pltpu.CompilerParams(
            vmem_limit_bytes=100 * 2**20,
            disable_semaphore_checks=True,
        ),
        name="adaln_decode",
    )(A_x, c, slabs(w_mod, 2), slabs(A_wq, 2), halves(A_k_cache), halves(A_v_cache),
      slabs(A_wo.T, 2), slabs(B_w3, 4), B_w4.T)
```
